```python
import os as _os
_os.environ.setdefault("JAX_PLATFORMS", "cpu")
import jax
import jax.numpy as jnp

def _softmax(x, axis=-1):
    return jax.nn.softmax(x, axis=axis)
def _gelu(x):
    return jax.nn.gelu(x, approximate=True)
def _silu(x):
    return jax.nn.silu(x)
def _sigmoid(x):
    return jax.nn.sigmoid(x)
def _layernorm(x, axis=-1, eps=1e-5):
    m = jnp.mean(x, axis=axis, keepdims=True)
    v = jnp.var(x, axis=axis, keepdims=True)
    return (x - m) / jnp.sqrt(v + eps)
def _scatter_add(tgt, idx, src, axis=0):
    return tgt.at[idx].add(src)
def _segment_sum(src, seg, n):
    return jax.ops.segment_sum(src, seg, n)
class _Rng:
    def __init__(self, key):
        self._k = key
    def _next(self):
        self._k, sub = jax.random.split(self._k)
        return sub
    def normal(self, shape):
        return jax.random.normal(self._next(), shape, dtype=jnp.bfloat16)
    def randint(self, lo, hi, shape):
        return jax.random.randint(self._next(), shape, lo, hi, dtype=jnp.int32)
    def uniform(self, shape, lo=0.0, hi=1.0):
        return jax.random.uniform(self._next(), shape, jnp.bfloat16, lo, hi)
    def permutation(self, n):
        return jax.random.permutation(self._next(), n)


kernel_name = 'gated_mix__softmax_full_mha__dense_activation_relu__prompt'

def setup_inputs():
    _rng = _Rng(jax.random.key(int.from_bytes(__import__("os").urandom(4), "little")))
    _w = (lambda a: (lambda t: t.astype(jnp.bfloat16) if jnp.issubdtype(t.dtype, jnp.floating) else t)(jnp.asarray(a)))
    def _A_setup():
        B, S, D = 1, 2048, 640
        return {
            "x": _w((lambda *s: _rng.normal(s) * 0.05)(B, S, D)),
            "wqkv": _w((lambda *s: _rng.normal(s) * 0.8)(D, 3 * D)),
            "wo": _w((lambda *s: _rng.normal(s) * 0.05)(D, D)),
        }
    _A_in = _A_setup()

    def _B_setup():
        B, S, D, Dff = 1, 2048, 640, 1536
        return {
            "x": _w((lambda *s: _rng.normal(s) * 0.05)(B, S, D)),
            "w1": _w((lambda *s: _rng.normal(s) * 0.05)(D, Dff)),
            "w2": _w((lambda *s: _rng.normal(s) * 0.05)(Dff, D)),
        }
    _B_in = _B_setup()

    return {
        "A_x": _A_in["x"],
        "A_wqkv": _A_in["wqkv"],
        "A_wo": _A_in["wo"],
        "B_x": _B_in["x"],
        "B_w1": _B_in["w1"],
        "B_w2": _B_in["w2"],
        "gate_w": _w((lambda *s: _rng.normal(s) * 0.05)(640) * 16.0),
    }

def reference(A_x, A_wqkv, A_wo, B_x, B_w1, B_w2, gate_w):
    def _A_ref(x, wqkv, wo):
        B, S, D = x.shape
        H = 32; Dh = D // H
        qkv = (lambda x, *d: x.transpose(*d))((x @ wqkv).reshape(B, S, 3, H, Dh), 2, 0, 3, 1, 4)
        q, k, v = qkv[0], qkv[1], qkv[2]
        scale = Dh ** -0.5
        scores = jnp.einsum("bhqd,bhkd->bhqk", q, k) * scale
        p = _softmax(scores, axis=-1)
        o = jnp.einsum("bhqk,bhkd->bhqd", p, v)
        return (lambda x, *d: x.transpose(*d))(o, 0, 2, 1, 3).reshape(B, S, D) @ wo

    def _B_ref(x, w1, w2):
        h = jnp.einsum("bsd,df->bsf", x, w1)
        zero = jnp.zeros_like(h)
        h = jnp.maximum(h, zero)
        return jnp.einsum("bsf,fd->bsd", h, w2)

    x = A_x
    g = _sigmoid((x * gate_w).sum(-1, keepdims=True))
    a = _A_ref(x, A_wqkv, A_wo)
    b = _B_ref(x, B_w1, B_w2)
    return g * a + (1 - g) * b
```

```python
import functools
import numpy as np
import jax
import jax.numpy as jnp
from jax import lax
import jax.experimental.pallas as pl
import jax.experimental.pallas.tpu as pltpu

S, D, H, DH, DFF = 2048, 640, 32, 20, 1536
NG = 6
F32, BF16 = jnp.float32, jnp.bfloat16
QSCALE = float(DH ** -0.5 * np.log2(np.e))

def make(QB=512, C=256, pipe=True, fallback=True):
    NQ = S // QB
    NC = S // C
    def kernel(x_ref, wqkv_ref, wo_ref, w1_ref, w2_ref, gw_ref, o_ref,
               k_s, qt_s, vt_s, ot_s, kmax_s, tmp_s):
        i = pl.program_id(0)

        @pl.when(i == 0)
        def _():
            lane = lax.broadcasted_iota(jnp.int32, (D, 128), 1)
            x = x_ref[...]
            wk = wqkv_ref[:, D:2 * D]
            lane2 = lax.broadcasted_iota(jnp.int32, (S, 128), 1)
            erow = lax.broadcasted_iota(jnp.int32, (8, 128), 0)
            elane = lax.broadcasted_iota(jnp.int32, (8, 128), 1)
            ind = jnp.where((elane >= erow * DH) & (elane < erow * DH + DH) & (erow < 6), 1.0, 0.0).astype(BF16)
            for g in range(NG):
                w = wqkv_ref[:, D + 120 * g: D + 120 * g + 128]
                nv = 120 if g < 5 else 40
                w = jnp.where(lane < nv, w, jnp.zeros_like(w))
                kg = jnp.dot(x, w, preferred_element_type=F32)
                kb = kg.astype(BF16)
                kf = kb.astype(F32)
                n2 = lax.dot_general(ind, (kf * kf).astype(BF16), (((1,), (1,)), ((), ())), preferred_element_type=F32)
                kmax_s[g] = jnp.broadcast_to(jnp.max(n2, axis=1, keepdims=True), (8, 128))
                k_s[g] = jnp.where(lane2 == 120, 1.0, kg).astype(BF16)
            qt = lax.dot_general(wqkv_ref[:, 0:D], x, (((0,), (1,)), ((), ())), preferred_element_type=F32)
            qt_s[0:D, :] = qt * QSCALE
            qt_s[D:, :] = jnp.zeros((768 - D, S), F32)
            vt = lax.dot_general(wqkv_ref[:, 2 * D:], x, (((0,), (1,)), ((), ())), preferred_element_type=F32)
            tmp_s[...] = vt
            row = lax.broadcasted_iota(jnp.int32, (24, S), 0)
            z8 = jnp.zeros((8, S), F32)
            for p in range(H // 2):
                ve = tmp_s[40 * p: 40 * p + 24, :]
                ve = jnp.where(row < 20, ve, jnp.where(row == 20, 1.0, 0.0))
                vt_s[2 * p] = jnp.concatenate([ve, z8], axis=0).astype(BF16)
                vo = tmp_s[40 * p + 16: 40 * p + 40, :]
                vo = jnp.where(row >= 4, vo, jnp.where(row == 0, 1.0, 0.0))
                vt_s[2 * p + 1] = jnp.concatenate([vo, z8], axis=0).astype(BF16)

        q0 = pl.multiple_of(i * QB, QB)
        row = lax.broadcasted_iota(jnp.int32, (128, QB), 0)
        r8 = lax.broadcasted_iota(jnp.int32, (8, QB), 0)
        r81 = lax.broadcasted_iota(jnp.int32, (8, 128), 0)

        def head(h, g, j, exact):
            qt = qt_s[pl.ds(pl.multiple_of(g * 120, 8), 128), pl.ds(q0, QB)]
            qt = jnp.where((row >= j * DH) & (row < j * DH + DH), qt, 0.0)
            if not exact:
                qn2 = jnp.sum(qt * qt, axis=0, keepdims=True)
                km = jnp.max(jnp.where(r81 == j, kmax_s[g], 0.0), axis=0, keepdims=True)
                km = jnp.concatenate([km] * (QB // 128), axis=1)
                m = jnp.sqrt(qn2 * km)
                qt = jnp.where(row == 120, -m, qt)
            qb = qt.astype(BF16)
            def qk(c):
                return jnp.dot(k_s[g, c * C:(c + 1) * C, :], qb, preferred_element_type=F32)
            def pv(c, p):
                return jnp.dot(vt_s[h, :, c * C:(c + 1) * C], p, preferred_element_type=F32)
            if exact:
                def mx(c, m):
                    s = jnp.dot(k_s[g, pl.ds(pl.multiple_of(c * C, C), C), :], qb, preferred_element_type=F32)
                    return jnp.maximum(m, jnp.max(s, axis=0, keepdims=True))
                m = lax.fori_loop(0, NC, mx, jnp.full((1, QB), -jnp.inf, F32))
                def ac(c, acc):
                    c0 = pl.multiple_of(c * C, C)
                    s = jnp.dot(k_s[g, pl.ds(c0, C), :], qb, preferred_element_type=F32)
                    p = jnp.exp2(s - m).astype(BF16)
                    return acc + jnp.dot(vt_s[h, :, pl.ds(c0, C)], p, preferred_element_type=F32)
                return lax.fori_loop(0, NC, ac, jnp.zeros((32, QB), F32))
            acc = None
            if pipe:
                p = jnp.exp2(qk(0)).astype(BF16)
                for c in range(NC):
                    if c + 1 < NC:
                        s = qk(c + 1)
                    r = pv(c, p)
                    acc = r if acc is None else acc + r
                    if c + 1 < NC:
                        p = jnp.exp2(s).astype(BF16)
            else:
                for c in range(NC):
                    r = pv(c, jnp.exp2(qk(c)).astype(BF16))
                    acc = r if acc is None else acc + r
            return acc

        def pair(p, lmin, exact):
            g = p // 3
            j = (p % 3) * 2
            ae = head(2 * p, g, j, exact)
            ao = head(2 * p + 1, g, j + 1, exact)
            le = ae[20:21, :]
            lo = ao[0:1, :]
            oe = ae[0:24] / le
            oo = ao[0:24] / lo
            mid = jnp.where(r8 < 4, oe[16:24], oo[0:8])
            ot_s[pl.ds(pl.multiple_of(p * 40, 8), 40), :] = jnp.concatenate([oe[0:16], mid, oo[8:24]], axis=0)
            ok = jnp.where((le >= 2.0 ** -30) & (lo >= 2.0 ** -30), 1.0, 0.0)
            return jnp.minimum(lmin, ok)

        ok = lax.fori_loop(0, H // 2, functools.partial(pair, exact=False), jnp.ones((1, QB), F32))
        if fallback:
            @pl.when(jnp.min(ok) < 0.5)
            def _():
                lax.fori_loop(0, H // 2, functools.partial(pair, exact=True), jnp.ones((1, QB), F32))

        xb = x_ref[pl.ds(q0, QB), :]
        a = lax.dot_general(ot_s[...].astype(BF16), wo_ref[...], (((0,), (0,)), ((), ())), preferred_element_type=F32)
        hh = jnp.maximum(jnp.dot(xb, w1_ref[...], preferred_element_type=F32), 0.0).astype(BF16)
        b = jnp.dot(hh, w2_ref[...], preferred_element_type=F32)
        gate = jax.nn.sigmoid(jnp.sum(xb.astype(F32) * gw_ref[...].astype(F32), axis=-1, keepdims=True))
        o_ref[...] = (gate * a + (1.0 - gate) * b).astype(o_ref.dtype)

    def fn(A_x, A_wqkv, A_wo, B_x, B_w1, B_w2, gate_w):
        full = lambda shp: pl.BlockSpec(shp, lambda i: (0,) * len(shp))
        out = pl.pallas_call(
            kernel,
            grid=(NQ,),
            in_specs=[full((S, D)), full((D, 3 * D)), full((D, D)), full((D, DFF)), full((DFF, D)), full((1, D))],
            out_specs=pl.BlockSpec((QB, D), lambda i: (i, 0)),
            out_shape=jax.ShapeDtypeStruct((S, D), BF16),
            scratch_shapes=[
                pltpu.VMEM((NG, S, 128), BF16),
                pltpu.VMEM((768, S), F32),
                pltpu.VMEM((H, 32, S), BF16),
                pltpu.VMEM((D, QB), F32),
                pltpu.VMEM((NG, 8, 128), F32),
                pltpu.VMEM((D, S), F32),
            ],
            compiler_params=pltpu.CompilerParams(dimension_semantics=("arbitrary",), vmem_limit_bytes=100 * 1024 * 1024),
            name="fused",
        )(A_x.reshape(S, D), A_wqkv, A_wo, B_w1, B_w2, gate_w.reshape(1, D))
        return out.reshape(1, S, D)
    return fn


_IMPL = make(**{'QB':512,'C':128})


@jax.jit
def pallas_gated_mix__softmax_full_mha__dense_activation_relu__prompt_kernel(
    A_x: jax.Array,
    A_wqkv: jax.Array,
    A_wo: jax.Array,
    B_x: jax.Array,
    B_w1: jax.Array,
    B_w2: jax.Array,
    gate_w: jax.Array,
):
    return _IMPL(A_x, A_wqkv, A_wo, B_x, B_w1, B_w2, gate_w)
```

```python
import numpy as np
import jax
import jax.numpy as jnp
from jax import lax
import jax.experimental.pallas as pl
import jax.experimental.pallas.tpu as pltpu

S, D, H, DH, DFF = 2048, 640, 32, 20, 1536
NP = H // 2
KD = 48
QB, C = 512, 128
NV = 16
NQ, NC, QT = S // QB, S // C, QB // 128
RA, RQ, RC = 512, 1024, 256
MP = 160
NA = S // RA
NSTEP = 2 * NQ * NC
F32, BF16, U32 = jnp.float32, jnp.bfloat16, jnp.uint32
QSCALE = float(DH ** -0.5 * np.log2(np.e))
BOUND_SLACK = 1.02
SUM_MIN, SUM_MAX = 2.0 ** -40, 2.0 * S
NN = (((1,), (0,)), ((), ()))
NT = (((1,), (1,)), ((), ()))


def _dot(a, b, dims=NN):
    return lax.dot_general(a, b, dims, precision=lax.Precision.DEFAULT, preferred_element_type=F32)


def _round(a):
    return a.astype(BF16).astype(F32)


def _rows(c, n):
    return pl.ds(pl.multiple_of(c * n, n), n)


def _kernel(x_hbm, wqkv_hbm, wo_hbm, w1_hbm, w2_hbm, gw_ref, o_hbm,
            x_s, wqkv_s, wo_s, w1_s, w2_s, o_s,
            km_s, wkt_s, wt_s, kt_s, k_s, q_s, qf_s, vt_s, ot_s, kb0, kb1, z_s,
            sem_x, sem_w, sem_o):
    kbs = (kb0, kb1)

    def xcopy(c):
        return pltpu.make_async_copy(x_hbm.at[_rows(c, RA), :], x_s.at[_rows(c, RA), :], sem_x.at[c])

    def wcopy(j):
        cs = pl.ds(j * D, D)
        return pltpu.make_async_copy(wqkv_hbm.at[:, cs], wqkv_s.at[:, cs], sem_w.at[j])

    def ocopy(c):
        return pltpu.make_async_copy(o_s.at[_rows(c, RC), :], o_hbm.at[_rows(c, RC), :], sem_o.at[c])

    wo_copy = pltpu.make_async_copy(wo_hbm, wo_s, sem_w.at[3])
    w1_copy = pltpu.make_async_copy(w1_hbm, w1_s, sem_w.at[4])
    w2_copy = pltpu.make_async_copy(w2_hbm, w2_s, sem_w.at[5])

    wcopy(1).start()
    xcopy(0).start()
    km_s[...] = jnp.zeros(km_s.shape, F32)

    def zinit(n, _):
        z_s[n] = 0
    lax.fori_loop(0, NSTEP, zinit, None)

    wcopy(1).wait()
    xcopy(1).start()
    for j in range(D // 128):
        wkt_s[128 * j:128 * (j + 1), :] = wqkv_s[:, D + 128 * j:D + 128 * (j + 1)].T
    ra8 = lax.broadcasted_iota(jnp.int32, (8, RA), 0)
    tpi = -(-10 // (NA - 1))

    def k_proj(c, _):
        xcopy(c).wait()

        @pl.when(c == 0)
        def _():
            wcopy(0).start()
            wcopy(2).start()

        @pl.when(c + 2 < NA)
        def _():
            xcopy(c + 2).start()

        @pl.when(c == 1)
        def _():
            wcopy(0).wait()
            wcopy(2).wait()

        r = _rows(c, RA)
        xc = x_s[r, :]
        for i in range(tpi):
            j = jnp.minimum((c - 1) * tpi + i, 9)
            src = jnp.where(c == 0, 5, jnp.where(j < 5, j, j + 5))
            dst = jnp.where(c == 0, 10, j)
            wt_s[_rows(dst, 128), :] = wqkv_s[:, _rows(src, 128)].T
        for m0 in range(0, D, MP):
            kt = _dot(wkt_s[m0:m0 + MP, :], xc, NT)
            kt_s[m0:m0 + MP, r] = _round(kt)
            for p in range(MP // 40):
                k2 = [kt[40 * p + 8 * t:40 * p + 8 * t + 8] for t in range(5)]
                k2 = [v * v for v in k2]
                for o, n2 in ((0, k2[0] + k2[1] + jnp.where(ra8 < 4, k2[2], 0.0)),
                              (1, k2[3] + k2[4] + jnp.where(ra8 < 4, 0.0, k2[2]))):
                    h = m0 // DH + 2 * p + o
                    n2 = jnp.sum(n2, axis=0, keepdims=True)
                    mx = km_s[h]
                    for l in range(RA // 128):
                        mx = jnp.maximum(mx, n2[:, 128 * l:128 * (l + 1)])
                    km_s[h] = mx
    lax.fori_loop(0, NA, k_proj, None)
    for h in range(H):
        km_s[h] = jnp.broadcast_to(jnp.max(km_s[h], axis=1, keepdims=True), (8, 128))

    wo_copy.start()
    w1_copy.start()
    w2_copy.start()
    r8 = lax.broadcasted_iota(jnp.int32, (8, RQ), 0)
    z8 = jnp.zeros((8, RQ), F32)
    cpr = RQ // C

    def qv_proj(c, _):
        r = _rows(c, RQ)
        xc = x_s[r, :]

        def put_k(p):
            kp = jnp.concatenate([kt_s[40 * p:40 * p + 40, r], jnp.where(r8 == 0, 1.0, 0.0)], axis=0).T
            k_s[p, r, :] = kp
            return kp

        k0 = put_k(0)
        todo = list(range(1, NP))
        for m0 in range(0, D, MP):
            for i in range(m0 * cpr // D, (m0 + MP) * cpr // D):
                for d in range(DH):
                    kb0[d, _rows(c * cpr + i, NV), :] = jnp.broadcast_to(
                        k0[(i + 1) * C - NV:(i + 1) * C, d:d + 1], (NV, 128))
            qt = _dot(wt_s[m0:m0 + MP, :], xc, NT) * QSCALE
            for pp in range(MP // 40):
                p = m0 // 40 + pp
                if pp % 2 == 0:
                    put_k(todo.pop(0))
                q = [qt[40 * pp + 8 * t:40 * pp + 8 * t + 8] for t in range(5)]
                for o in range(2):
                    h = 2 * p + o
                    mid = jnp.where(r8 < 4, q[2], 0.0) if o == 0 else jnp.where(r8 < 4, 0.0, q[2])
                    qa, qb = (q[0], q[1]) if o == 0 else (q[3], q[4])
                    n2 = jnp.sum(qa * qa + qb * qb + mid * mid, axis=0, keepdims=True)
                    shift = -BOUND_SLACK * jnp.sqrt(n2 * jnp.concatenate([km_s[h]] * (RQ // 128), axis=1))
                    tile = [qa, qb, mid, z8, z8] if o == 0 else [z8, z8, mid, qa, qb]
                    tile.append(jnp.where(r8 == 0, shift, 0.0))
                    q_s[h, :, r] = pltpu.bitcast(jnp.concatenate(tile, axis=0).astype(BF16), U32)
                    qf = ([qa, qb, jnp.where(r8 < 4, q[2], shift)] if o == 0
                          else [jnp.where(r8 < 4, shift, q[2]), qa, qb])
                    qf_s[h, :, r] = _round(jnp.concatenate(qf, axis=0))
        for m0 in range(0, D, MP):
            vt = _round(_dot(wt_s[D + m0:D + m0 + MP, :], xc, NT))
            for pp in range(MP // 40):
                p = m0 // 40 + pp
                if pp % 2 == 0 and todo:
                    put_k(todo.pop(0))
                v = [vt[40 * pp + 8 * t:40 * pp + 8 * t + 8] for t in range(5)]
                ve = [v[0], v[1], jnp.where(r8 < 4, v[2], jnp.where(r8 == 4, 1.0, 0.0))]
                vo = [jnp.where(r8 >= 4, v[2], jnp.where(r8 == 0, 1.0, 0.0)), v[3], v[4]]
                vt_s[2 * p, :, r] = jnp.concatenate(ve, axis=0)
                vt_s[2 * p + 1, :, r] = jnp.concatenate(vo, axis=0)
    lax.fori_loop(0, S // RQ, qv_proj, None)

    rq8 = lax.broadcasted_iota(jnp.int32, (8, QB), 0)

    def attend(p, safe):
        steps = [(e, u, c) for e in range(2) for u in range(NQ) for c in range(NC)]
        never = lax.broadcasted_iota(jnp.int32, (8, 128), 0) < z_s[0]
        never24 = lax.broadcasted_iota(jnp.int32, (24, QB), 0) < z_s[0]
        nrow = (C - NV) // 8
        probs, acc, vpu = {}, {}, {}

        def vpu_scores(n):
            e, u, c = steps[n]
            z = z_s[n]

            def qrow(d, l):
                row = d if e == 0 else (d + 4 if d < DH else 0)
                lanes = slice(u * QB + 128 * l, u * QB + 128 * (l + 1))
                return jnp.broadcast_to(qf_s[2 * p + e + z, row:row + 1, lanes], (8, 128))

            shift = [qrow(DH, l) for l in range(QT)]
            res = [list(shift) for _ in range(NV // 8)]
            partial = []
            for d in range(DH):
                kk = [kbs[e][d + z, c * NV + 8 * i:c * NV + 8 * i + 8, :] for i in range(NV // 8)]
                now = []
                for l in range(QT):
                    qq = qrow(d, l)
                    for i in range(NV // 8):
                        res[i][l] = res[i][l] + kk[i] * qq
                        now.append(res[i][l])
                partial += [now] * len(now)
            vpu["partial"], vpu["used"] = partial, 0
            vpu["probs"] = [jnp.exp2(jnp.concatenate(r, axis=1)) for r in res]

        def paced(v):
            partial, j = vpu["partial"], vpu["used"]
            vpu["used"] += 1
            now = partial[(j + 1) * len(partial) // (nrow + 3) - 1]
            w = v.shape[1]
            return jnp.where(never[:, :w], now[j % len(now)][:, :w], v)

        def scores(n):
            e, u, c = steps[n]
            z = z_s[n]
            order = list(range(nrow))[::-1]
            keys = jnp.concatenate([paced(k_s[p + z, c * C + 8 * j:c * C + 8 * j + 8, :]) for j in order], axis=0)
            sc = _dot(keys, pltpu.bitcast(q_s[2 * p + e + z, :, u * QB:(u + 1) * QB], BF16))
            probs[n] = jnp.concatenate([jnp.exp2(sc[8 * j:8 * j + 8]) for j in order] + vpu["probs"], axis=0)

        def values(n):
            e, u, c = steps[n]
            v = vt_s[2 * p + e + z_s[n], :, c * C:(c + 1) * C]
            if n + 2 < NSTEP:
                v = jnp.concatenate([paced(v[8 * i:8 * i + 8]) for i in range(3)], axis=0)
            r = _dot(v, probs.pop(n))
            if c > 0:
                r = acc[e, u] + r
            elif n > 0:
                r = jnp.where(never24, acc[steps[n - 1][:2]], r)
            acc[e, u] = r
            if c == NC - 1:
                ot_s[2 * p + e, :, u * QB:(u + 1) * QB] = r

        vpu_scores(0)
        for n in range(NSTEP + 1):
            if n < NSTEP:
                scores(n)
            if n + 1 < NSTEP:
                vpu_scores(n + 1)
            if n >= 1:
                values(n - 1)
            if n < NSTEP and n % NQ == 0:
                e, c = 1 - n // (NQ * NC), n % (NQ * NC) // NQ
                kk = k_s[p if e == 1 else jnp.minimum(p + 1, NP - 1), (c + 1) * C - NV:(c + 1) * C, :]
                for d in range(DH):
                    kbs[e][d, c * NV:(c + 1) * NV, :] = jnp.broadcast_to(
                        kk[:, DH * e + d:DH * e + d + 1], (NV, 128))
        for (e, u), a in acc.items():
            sums = a[16:24] if e == 0 else a[0:8]
            ok = jnp.where(sums >= SUM_MIN, jnp.where(sums <= SUM_MAX, 1.0, 0.0), 0.0)
            safe = jnp.minimum(safe, jnp.where(rq8 == 4 - 4 * e, ok, 1.0))
        return safe

    safe = lax.fori_loop(0, NP, attend, jnp.ones((8, QB), F32))

    @pl.when(jnp.min(safe) < 0.5)
    def _():
        ce = 256
        rowq = lax.broadcasted_iota(jnp.int32, (KD, QB), 0)

        def attend_true_max(t, _):
            qs = _rows(t // H, QB)
            h = t % H
            q = pltpu.bitcast(q_s[h, :, qs], BF16)
            q = jnp.where(rowq == 40, jnp.zeros_like(q), q)

            def sc(c):
                return _dot(k_s[h // 2, _rows(c, ce), :], q)

            m = lax.fori_loop(0, S // ce, lambda c, m: jnp.maximum(m, jnp.max(sc(c), axis=0, keepdims=True)),
                              jnp.full((1, QB), -jnp.inf, F32))

            def add(c, acc):
                return acc + _dot(vt_s[h, :, _rows(c, ce)], jnp.exp2(sc(c) - m).astype(BF16))
            ot_s[h, :, qs] = lax.fori_loop(0, S // ce, add, jnp.zeros((24, QB), F32))
        lax.fori_loop(0, NQ * H, attend_true_max, None)

    wo_copy.wait()
    w1_copy.wait()
    w2_copy.wait()
    gw = gw_ref[...].astype(F32).reshape(1, D)
    rc8 = lax.broadcasted_iota(jnp.int32, (8, RC), 0)

    def mix(c, _):
        r = _rows(c, RC)
        xb = x_s[r, :]
        hidden = jnp.maximum(_dot(xb, w1_s[...]), 0.0).astype(BF16)
        parts = []
        for p in range(NP):
            ae = ot_s[2 * p, :, r]
            ao = ot_s[2 * p + 1, :, r]
            oe = ae * (1.0 / ae[20:21])
            oo = ao * (1.0 / ao[0:1])
            parts += [oe[0:16], jnp.where(rc8 < 4, oe[16:24], oo[0:8]), oo[8:24]]
        a = _dot(jnp.concatenate(parts, axis=0).T.astype(BF16), wo_s[...])
        b = _dot(hidden, w2_s[...])
        gate = jax.nn.sigmoid(jnp.sum(xb.astype(F32) * gw, axis=-1, keepdims=True))
        o_s[r, :] = (gate * a + (1.0 - gate) * b).astype(o_s.dtype)
        ocopy(c).start()
    lax.fori_loop(0, S // RC, mix, None)
    for c in range(S // RC):
        ocopy(c).wait()


@jax.jit
def pallas_gated_mix__softmax_full_mha__dense_activation_relu__prompt_kernel(
    A_x: jax.Array,
    A_wqkv: jax.Array,
    A_wo: jax.Array,
    B_x: jax.Array,
    B_w1: jax.Array,
    B_w2: jax.Array,
    gate_w: jax.Array,
):
    del B_x
    hbm = pl.BlockSpec(memory_space=pl.ANY)
    vmem = pltpu.VMEM
    out = pl.pallas_call(
        _kernel,
        in_specs=[hbm] * 5 + [pl.BlockSpec(memory_space=pltpu.VMEM)],
        out_specs=hbm,
        out_shape=jax.ShapeDtypeStruct((S, D), BF16),
        scratch_shapes=[
            vmem((S, D), BF16), vmem((D, 3 * D), BF16), vmem((D, D), BF16),
            vmem((D, DFF), BF16), vmem((DFF, D), BF16), vmem((S, D), BF16),
            vmem((H, 8, 128), F32),
            vmem((D, D), BF16), vmem((2 * D + 128, D), BF16),
            vmem((D, S), F32), vmem((NP, S, KD), F32),
            vmem((H, KD // 2, S), U32), vmem((H, 24, S), F32),
            vmem((H, 24, S), F32), vmem((H, 24, S), F32),
            vmem((DH, NC * NV, 128), F32), vmem((DH, NC * NV, 128), F32),
            pltpu.SMEM((NSTEP,), jnp.int32),
            pltpu.SemaphoreType.DMA((NA,)), pltpu.SemaphoreType.DMA((6,)),
            pltpu.SemaphoreType.DMA((S // RC,)),
        ],
        compiler_params=pltpu.CompilerParams(vmem_limit_bytes=100 * 1024 * 1024),
        name="fused",
    )(A_x.reshape(S, D), A_wqkv, A_wo, B_w1, B_w2, gate_w)
    return out.reshape(1, S, D)
```
